```python
import jax
import jax.numpy as jnp

def _softmax(x, axis=-1):
    return jax.nn.softmax(x, axis=axis)
def _gelu(x):
    return jax.nn.gelu(x, approximate=True)
def _silu(x):
    return jax.nn.silu(x)
def _sigmoid(x):
    return jax.nn.sigmoid(x)
def _layernorm(x, axis=-1, eps=1e-5):
    m = jnp.mean(x, axis=axis, keepdims=True)
    v = jnp.var(x, axis=axis, keepdims=True)
    return (x - m) / jnp.sqrt(v + eps)
def _scatter_add(tgt, idx, src, axis=0):
    return tgt.at[idx].add(src)
def _segment_sum(src, seg, n):
    return jax.ops.segment_sum(src, seg, n)
class _Rng:
    def __init__(self, key):
        self._k = key
    def _next(self):
        self._k, sub = jax.random.split(self._k)
        return sub
    def normal(self, shape):
        return jax.random.normal(self._next(), shape, dtype=jnp.bfloat16)
    def randint(self, lo, hi, shape):
        return jax.random.randint(self._next(), shape, lo, hi, dtype=jnp.int32)
    def uniform(self, shape, lo=0.0, hi=1.0):
        return jax.random.uniform(self._next(), shape, jnp.bfloat16, lo, hi)
    def permutation(self, n):
        return jax.random.permutation(self._next(), n)


kernel_name = 'sequential_preLN__sliding_block_cached__moe_arch_mod__decode'

def setup_inputs():
    _rng = _Rng(jax.random.key(int.from_bytes(__import__("os").urandom(4), "little")))
    _w = (lambda a: (lambda t: t.astype(jnp.bfloat16) if jnp.issubdtype(t.dtype, jnp.floating) else t)(jnp.asarray(a)))
    def _A_setup():
        B, Sq, D = 1, 1, 640
        Hq, Hkv, Sk, Dh = 32, 32, 32768, 192
        assert Hq % Hkv == 0, (Hq, Hkv)
        return {
            "x": _w((lambda *s: _rng.normal(s) * 0.05)(B, Sq, D)),
            "k_cache": _w((lambda *s: _rng.normal(s) * 0.05)(B, Hkv, Sk, Dh)),
            "v_cache": _w((lambda *s: _rng.normal(s) * 0.05)(B, Hkv, Sk, Dh)),
            "wq": _w((lambda *s: _rng.normal(s) * 0.05)(D, Hq * Dh) * (D ** -0.5)),
            "wo": _w((lambda *s: _rng.normal(s) * 0.05)(Hq * Dh, D) * ((Hq * Dh) ** -0.5)),
        }
    _A_in = _A_setup()

    def _B_setup():
        B, S, D, F, C = 1, 1, 640, 1536, 1
        return {
            "x": _w((lambda *s: _rng.normal(s) * 0.05)(B, S, D)),
            "w_r": _w((lambda *s: _rng.normal(s) * 0.05)(D)),
            "w_gate": _w((lambda *s: _rng.normal(s) * 0.05)(D, F)),
            "w_up": _w((lambda *s: _rng.normal(s) * 0.05)(D, F)),
            "w_down": _w((lambda *s: _rng.normal(s) * 0.05)(F, D)),
        }
    _B_in = _B_setup()

    return {
        "A_x": _A_in["x"],
        "A_k_cache": _A_in["k_cache"],
        "A_v_cache": _A_in["v_cache"],
        "A_wq": _A_in["wq"],
        "A_wo": _A_in["wo"],
        "B_x": _B_in["x"],
        "B_w_r": _B_in["w_r"],
        "B_w_gate": _B_in["w_gate"],
        "B_w_up": _B_in["w_up"],
        "B_w_down": _B_in["w_down"],
    }

def reference(A_x, A_k_cache, A_v_cache, A_wq, A_wo, B_x, B_w_r, B_w_gate, B_w_up, B_w_down):
    def _A_ref(x, k_cache, v_cache, wq, wo):
        B, Sq, D = x.shape
        Hq, Dh = 32, 192
        Hkv, Sk = k_cache.shape[1], k_cache.shape[2]
        W = min(4096, max(256, Sk // 4))
        rep = Hq // Hkv
        q = (lambda x, *d: x.transpose(*d))((x @ wq).reshape(B, Sq, Hq, Dh), 0, 2, 1, 3)
        k = jnp.repeat(k_cache[:, :, Sk - W:, :], rep, axis=1)
        v = jnp.repeat(v_cache[:, :, Sk - W:, :], rep, axis=1)
        scores = jnp.einsum("bhqd,bhkd->bhqk", q, k) * (Dh ** -0.5)
        p = _softmax(scores, axis=-1)
        o = jnp.einsum("bhqk,bhkd->bhqd", p, v)
        return (lambda x, *d: x.transpose(*d))(o, 0, 2, 1, 3).reshape(B, Sq, Hq * Dh) @ wo

    def _B_ref(x, w_r, w_gate, w_up, w_down):
        B, S, D = x.shape
        C = 1
        r = x @ w_r
        idx = jnp.argsort(-r, axis=-1)[:, :C]
        idx_e = jnp.repeat(idx.reshape(B, C, 1), D, axis=2)
        x_sel = jnp.take_along_axis(x, idx_e, axis=1)
        g = _silu(x_sel @ w_gate)
        u = x_sel @ w_up
        y = (g * u) @ w_down
        r_sel = _sigmoid(jnp.take_along_axis(r, idx, axis=1))
        y = y * r_sel.reshape(B, C, 1)
        b_off = (jnp.arange(B) * S).reshape(B, 1)
        flat_idx = (idx + b_off).reshape(B * C)
        zero = (x * 0.0).reshape(B * S, D)
        upd = _scatter_add(zero, flat_idx, y.reshape(B * C, D), axis=0)
        return x + upd.reshape(B, S, D)

    x = A_x
    h = x + _A_ref(_layernorm(x, axis=-1), A_k_cache, A_v_cache, A_wq, A_wo)
    h2 = h + _B_ref(_layernorm(h, axis=-1), B_w_r, B_w_gate, B_w_up, B_w_down)
    return h2
```

```python
import functools
import jax
import jax.numpy as jnp
from jax import lax
import jax.experimental.pallas as pl
import jax.experimental.pallas.tpu as pltpu

EPS = 1e-5
NBUF = 4
KV_ROWS = 64
KV_ROWS_Q1 = 56
KV_COLS = 512
QO_SLABS, QO_GROUP, QO_ROWS = 15, 3, 32
GU_SLABS = 4
WD_SLABS = 3
LAST = 8

f32, bf16 = jnp.float32, jnp.bfloat16


def _layernorm(x):
    m = jnp.mean(x, axis=-1, keepdims=True)
    d = x - m
    v = jnp.mean(d * d, axis=-1, keepdims=True)
    return d / jnp.sqrt(v + EPS)


def _column(row):
    return jnp.broadcast_to(row, (128, 128)).T


def _aligned(i, n):
    return i if isinstance(i, int) else pl.multiple_of(i, n)


def _kernel(x_hbm, k_hbm, v_hbm, wq_hbm, wo_hbm, wr_hbm, wg_hbm, wu_hbm, wd_hbm,
            o_ref,
            x_s, wr_s, wq_s, wo_s, wg_s, wu_s, wd_s, k_s, v_s, xc_s, qt_s, q_s, p_s, acc_s, sems):
    _, Dh, W = k_s.shape
    H = k_hbm.shape[0] // Dh
    Sk = k_hbm.shape[1]
    D = x_hbm.shape[-1]
    F = wg_hbm.shape[-1]
    DT = D // 128
    S_K, S_V = 0, NBUF
    S_X, S_R, S_Q, S_O, S_G, S_U, S_D = range(2 * NBUF, 2 * NBUF + 7)

    def copy(src, dst, sem, queue):
        pltpu.make_async_copy(src, dst, sems.at[sem]).start(priority=queue)

    def done(dst, sem):
        pltpu.make_async_copy(dst, dst, sems.at[sem]).wait()

    NR = Dh // KV_ROWS
    NC = W // KV_COLS
    LAG = NR * NC

    def kv(src, dst, sem, h):
        buf = h % NBUF

        def start(c, r, queue):
            r0, n = ((r * KV_ROWS, KV_ROWS_Q1) if queue
                     else (r * KV_ROWS + KV_ROWS_Q1, KV_ROWS - KV_ROWS_Q1))
            col = _aligned(c * KV_COLS, KV_COLS)
            copy(src.at[pl.ds(_aligned(h * Dh + r0, 8), n),
                        pl.ds(_aligned(Sk - W + col, KV_COLS), KV_COLS)],
                 dst.at[buf, pl.ds(r0, n), pl.ds(col, KV_COLS)], sem + buf, queue)
        return start

    K = functools.partial(kv, k_hbm, k_s, S_K)
    V = functools.partial(kv, v_hbm, v_s, S_V)

    NG = QO_SLABS // QO_GROUP
    NQO = NG * wq_hbm.shape[1] // QO_ROWS

    def qo(i, queue):
        src, dst, sem = (wq_hbm, wq_s, S_Q) if queue else (wo_hbm, wo_s, S_O)
        idx = (pl.ds(QO_GROUP * (i % NG), QO_GROUP),
               pl.ds(_aligned(QO_ROWS * (i // NG), QO_ROWS), QO_ROWS))
        copy(src.at[idx], dst.at[idx], sem, queue)

    NF = F // 512
    NGU = wg_hbm.shape[1] // 8 * NF

    def gu(i, queue):
        src, dst, sem = (wg_hbm, wg_s, S_G) if queue else (wu_hbm, wu_s, S_U)
        idx = (slice(None), pl.ds(_aligned(8 * (i // NF), 8), 8),
               pl.ds(_aligned(512 * (i % NF), 512), 512))
        copy(src.at[idx], dst.at[idx], sem, queue)

    DR = wd_hbm.shape[1]
    NWD = DR // 8
    NB = DR // 128

    def wd(i, queue):
        sem = S_D + i // 16
        if queue:
            sem = jnp.where(i < NWD - LAST, sem, S_D + NB + i - (NWD - LAST))
        idx = (pl.ds(0, WD_SLABS - 1) if queue else pl.ds(WD_SLABS - 1, 1),
               pl.ds(_aligned(8 * i, 8), 8))
        copy(wd_hbm.at[idx], wd_s.at[idx], sem, queue)

    def stream(n, y=None, y0=0, x=None, x0=0):
        def body(t, carry):
            if y is not None:
                y(y0 + t, 1)
            if x is not None:
                x(x0 + t, 0)
            return carry
        if n > 0:
            lax.fori_loop(0, n, body, 0)

    def stream_matrix(y, x):
        def body(c, carry):
            for r in range(NR):
                y(c, r, 1)
                x(c, r, 0)
            return carry
        lax.fori_loop(0, NC, body, 0)

    def by_block(phase, first):
        return lambda c, r, queue: phase(first + c * NR + r, queue)

    QT = H * Dh // 128
    TR = wq_s.shape[1]

    def project(g):
        def band(b, acc):
            row = (b * QT + 16 * g) * 8
            w = wq_s[row // TR, pl.ds(pl.multiple_of(row % TR, 128), 128), :]
            m = xc_s[pl.ds(pl.multiple_of(b * 8, 8), 8), :]
            return tuple(a + w[8 * j:8 * j + 8].astype(f32) * m for j, a in enumerate(acc))
        acc = lax.fori_loop(0, D // 8, band, tuple(jnp.zeros((8, 128), f32) for _ in range(16)),
                            unroll=2)
        for j in range(16):
            qt_s[:, pl.ds(_aligned((16 * g + j) * 128, 128), 128)] = jnp.broadcast_to(
                jnp.sum(acc[j], axis=0, keepdims=True), (8, 128))

    def scores(h):
        buf = h % NBUF
        done(k_s.at[buf], S_K + buf)
        s = jnp.dot(q_s[h].astype(bf16), k_s[buf], preferred_element_type=f32) * Dh ** -0.5
        m = jnp.max(s, axis=-1, keepdims=True)
        e = jnp.exp(s - m)
        p_s[...] = e * (1.0 / jnp.sum(e, axis=-1, keepdims=True))

    def values(h):
        buf = h % NBUF
        done(v_s.at[buf], S_V + buf)
        acc = [acc_s[:, t * 128:(t + 1) * 128] for t in range(DT)]
        for r in range(Dh // 16):
            a0 = jnp.zeros((8, 128), f32)
            a1 = jnp.zeros((8, 128), f32)
            for j in range(W // 128):
                vv = v_s[buf, r * 16:(r + 1) * 16, j * 128:(j + 1) * 128].astype(f32)
                pp = p_s[:, j * 128:(j + 1) * 128]
                a0 = a0 + vv[:8] * pp
                a1 = a1 + vv[8:] * pp
            o = (jnp.sum(a0, axis=-1, keepdims=True), jnp.sum(a1, axis=-1, keepdims=True))
            for t in range(DT):
                row = (h * Dh + r * 16) * DT + 16 * t
                ww = wo_s[row // TR, pl.ds(_aligned(row % TR, 16), 16), :].astype(f32)
                for half in range(2):
                    band, col = divmod(2 * t + half, DT)
                    acc[col] = acc[col] + ww[8 * half:8 * half + 8] * o[band]
        for t in range(DT):
            acc_s[:, t * 128:(t + 1) * 128] = acc[t]

    x_cp = pltpu.make_async_copy(x_hbm, x_s, sems.at[S_X])
    wr_cp = pltpu.make_async_copy(wr_hbm, wr_s, sems.at[S_R])
    stream(LAG, y=qo)
    x_cp.start()
    wr_cp.start()
    stream(NQO - LAG, y=qo, y0=LAG, x=qo)
    x_cp.wait()
    wr_cp.wait()
    x = x_s[0].astype(f32)
    xn = _layernorm(x).astype(bf16).astype(f32)
    for t in range(DT):
        xc_s[t * 128:(t + 1) * 128, :] = _column(xn[:, t * 128:(t + 1) * 128])
    acc_s[...] = jnp.zeros_like(acc_s)
    stream_matrix(K(0), by_block(qo, NQO - LAG))

    def step(h, carry):
        @pl.when(h < H)
        def _():
            stream_matrix(V(h), K(h))

        @pl.when(h == H)
        def _():
            stream(LAG, y=gu, y0=LAG, x=gu)

        @pl.when(h == 0)
        def _():
            done(wq_s, S_Q)

        @pl.when(h < 2)
        def _():
            project(2 * h)

        @pl.when(h >= 2)
        def _():
            scores(h - 2)

        @pl.when(h < H - 1)
        def _():
            stream_matrix(K(h + 1), V(h))

        @pl.when(h == H - 1)
        def _():
            stream_matrix(by_block(gu, 0), V(h))

        @pl.when(h == H)
        def _():
            stream(NGU - 2 * LAG, y=gu, y0=2 * LAG, x=gu, x0=LAG)
            stream(3 * LAG - NGU, y=wd, x=gu, x0=NGU - LAG)

        @pl.when(h == 0)
        def _():
            project(1)

        @pl.when(h == 1)
        def _():
            for c in range(H // 2):
                q2 = qt_s[:, c * 2 * Dh:(c + 1) * 2 * Dh]
                q_s[2 * c] = q2[:, :Dh]
                q_s[2 * c + 1] = q2[:, Dh:]
            done(wo_s, S_O)

        @pl.when(h >= 2)
        def _():
            values(h - 2)
        return carry

    lax.fori_loop(0, H + 1, step, 0)
    stream(NGU - 2 * LAG, y=wd, y0=3 * LAG - NGU, x=gu, x0=2 * LAG)
    scores(H - 1)

    def stream_down(lo, hi):
        both = max(min(hi, NWD - LAG) - lo, 0)
        stream(both, y=wd, y0=LAG + lo, x=wd, x0=lo)
        stream(hi - lo - both, x=wd, x0=lo + both)

    stream_down(0, 12)
    values(H - 1)

    hres = x + jnp.sum(acc_s[...], axis=0, keepdims=True)
    hn = _layernorm(hres)
    wr = wr_s[...].astype(f32).reshape(1, D)
    gate = jax.nn.sigmoid(jnp.sum(hn * wr, axis=-1, keepdims=True))
    hb = jnp.broadcast_to(hn, (8, D)).astype(bf16)

    stream_down(12, 36)
    done(wg_s, S_G)
    done(wu_s, S_U)
    act = []
    for c, (lo, hi) in enumerate(((36, 48), (48, NWD), (NWD, NWD))):
        cs = slice(c * DR, (c + 1) * DR)
        g = jnp.dot(hb, wg_s[:, :, cs].reshape(D, DR), preferred_element_type=f32)
        u = jnp.dot(hb, wu_s[:, :, cs].reshape(D, DR), preferred_element_type=f32)
        act.append((g * jax.nn.sigmoid(g) * u).astype(bf16))
        stream_down(lo, hi)

    def down(g, lo, hi):
        return jnp.dot(act[g][:, lo:hi], wd_s[g, lo:hi, :], preferred_element_type=f32)

    y = jnp.zeros((8, D), f32)
    for c in range(NB - 1):
        done(wd_s.at[:, pl.ds(c * 128, 128)], S_D + c)
        for g in range(WD_SLABS):
            y = y + down(g, c * 128, (c + 1) * 128)
    mid, end = DR - 128, DR - 8 * LAST
    cols = [_column(act[g][:1, mid:].astype(f32) * gate) for g in range(WD_SLABS - 1)]
    done(wd_s.at[WD_SLABS - 1, pl.ds(mid, 128)], S_D + NB - 1)
    done(wd_s.at[pl.ds(0, WD_SLABS - 1), pl.ds(mid, end - mid)], S_D + NB - 1)
    y = y + down(WD_SLABS - 1, mid, DR)
    for g in range(WD_SLABS - 1):
        y = y + down(g, mid, end)
    base = hres + (hn + y[:1] * gate)
    first = lax.broadcasted_iota(jnp.int32, (8, 128), 0) == 0
    a = [jnp.where(first, base[:, j * 128:(j + 1) * 128], 0.0) for j in range(DT)]
    for t in range(LAST):
        r0 = end + 8 * t
        done(wd_s.at[pl.ds(0, WD_SLABS - 1), pl.ds(r0, 8)], S_D + NB + t)
        for g in range(WD_SLABS - 1):
            w = wd_s[g, r0:r0 + 8, :].astype(f32)
            m = cols[g][r0 - mid:r0 - mid + 8]
            a = [a[j] + w[:, j * 128:(j + 1) * 128] * m for j in range(DT)]
    out = jnp.sum(jnp.concatenate(a, axis=1), axis=0, keepdims=True)
    o_ref[0] = out.astype(o_ref.dtype)


def _tiles(a):
    R, C = a.shape
    return a.reshape(R // 8, 8, C // 128, 128).transpose(0, 2, 1, 3).reshape(R * C // 128, 128)


def _slabs(a, n):
    return a.reshape(n, a.shape[0] // n, a.shape[1])


@jax.jit
def pallas_sequential_preLN__sliding_block_cached__moe_arch_mod__decode_kernel(
    A_x: jax.Array,
    A_k_cache: jax.Array,
    A_v_cache: jax.Array,
    A_wq: jax.Array,
    A_wo: jax.Array,
    B_x: jax.Array,
    B_w_r: jax.Array,
    B_w_gate: jax.Array,
    B_w_up: jax.Array,
    B_w_down: jax.Array,
):
    del B_x
    _, H, Sk, Dh = A_k_cache.shape
    D = A_x.shape[-1]
    W = min(4096, max(256, Sk // 4))
    kt = jnp.transpose(A_k_cache, (0, 1, 3, 2)).reshape(H * Dh, Sk)
    vt = jnp.transpose(A_v_cache, (0, 1, 3, 2)).reshape(H * Dh, Sk)
    wq, wo = _slabs(_tiles(A_wq), QO_SLABS), _slabs(_tiles(A_wo), QO_SLABS)
    wg, wu = _slabs(B_w_gate, GU_SLABS), _slabs(B_w_up, GU_SLABS)
    wd = _slabs(B_w_down, WD_SLABS)
    like = lambda a: pltpu.VMEM(a.shape, a.dtype)
    return pl.pallas_call(
        _kernel,
        out_shape=jax.ShapeDtypeStruct(A_x.shape, A_x.dtype),
        in_specs=[pl.BlockSpec(memory_space=pl.ANY)] * 9,
        scratch_shapes=[
            like(A_x), like(B_w_r), like(wq), like(wo), like(wg), like(wu), like(wd),
            pltpu.VMEM((NBUF, Dh, W), A_k_cache.dtype),
            pltpu.VMEM((NBUF, Dh, W), A_v_cache.dtype),
            pltpu.VMEM((D, 128), f32),
            pltpu.VMEM((8, H * Dh), f32),
            pltpu.VMEM((H, 8, Dh), f32),
            pltpu.VMEM((8, W), f32),
            pltpu.VMEM((8, D), f32),
            pltpu.SemaphoreType.DMA((2 * NBUF + 6 + wd.shape[1] // 128 + LAST,)),
        ],
        compiler_params=pltpu.CompilerParams(
            vmem_limit_bytes=100 * 2**20,
            disable_bounds_checks=True,
            disable_semaphore_checks=True),
    )(A_x, kt, vt, wq, wo, B_w_r, wg, wu, wd)
```

```python
import functools
import jax
import jax.numpy as jnp
from jax import lax
import jax.experimental.pallas as pl
import jax.experimental.pallas.tpu as pltpu

EPS = 1e-5
NBUF = 4
KV_ROWS = (16, 48)
COLS = 512
QO_SLABS, QO_GROUP, QO_ROWS = 15, 3, 32
GU_SLABS = 4
WD_SLABS = 3
LAST, LAST_ROWS = 8, 16

f32, bf16 = jnp.float32, jnp.bfloat16


def _layernorm(x):
    m = jnp.mean(x, axis=-1, keepdims=True)
    d = x - m
    v = jnp.mean(d * d, axis=-1, keepdims=True)
    return d / jnp.sqrt(v + EPS)


def _column(row):
    return jnp.broadcast_to(row, (128, 128)).T


def _aligned(i, n):
    return i if isinstance(i, int) else pl.multiple_of(i, n)


class _Phase:
    def __init__(self, rounds, width, start):
        self.width, self.start, self.slots = width, start, rounds * width

    def start_slot(self, i, queue):
        self.start(i // self.width, i % self.width, queue)


def _stream(n, q1=None, first1=0, q0=None, first0=0):
    if n <= 0:
        return
    lanes = [(p, first, queue) for p, first, queue in ((q1, first1, 1), (q0, first0, 0)) if p]
    width = max(p.width for p, _, _ in lanes)
    assert n % width == 0
    assert all(width % p.width == 0 and first % p.width == 0 and first + n <= p.slots
               for p, first, _ in lanes)

    def body(t, carry):
        for j in range(width):
            for p, first, queue in lanes:
                p.start(first // p.width + t * (width // p.width) + j // p.width, j % p.width, queue)
        return carry

    lax.fori_loop(0, n // width, body, 0)


def _kernel(x_hbm, k_hbm, v_hbm, wq_hbm, wo_hbm, wr_hbm, wg_hbm, wu_hbm, wd_hbm,
            o_ref,
            x_s, wr_s, wq_s, wo_s, wg_s, wu_s, wd_s, k_s, v_s, xc_s, qt_s, q_s, p_s, acc_s, sems):
    _, Dh, W = k_s.shape
    H = k_hbm.shape[0] // Dh
    Sk = k_hbm.shape[1]
    D = x_hbm.shape[-1]
    DT = D // 128
    S_K, S_V = 0, NBUF
    S_X, S_R, S_Q, S_O, S_G, S_U, S_D = range(2 * NBUF, 2 * NBUF + 7)

    def copy(src, dst, sem, queue):
        pltpu.make_async_copy(src, dst, sems.at[sem]).start(priority=queue)

    def done(dst, sem):
        pltpu.make_async_copy(dst, dst, sems.at[sem]).wait()

    groups = Dh // sum(KV_ROWS)

    def head_matrix(src, dst, sem, h):
        buf = h & (NBUF - 1)

        def start(c, g, queue):
            n = KV_ROWS[queue]
            r0 = g * n if queue else groups * KV_ROWS[1] + g * n
            col = _aligned(((c & ~3) | (-c & 3)) * COLS, COLS)
            copy(src.at[pl.ds(_aligned(h * Dh + r0, 8), n), pl.ds(_aligned(Sk - W + col, COLS), COLS)],
                 dst.at[buf, pl.ds(r0, n), pl.ds(col, COLS)], sem + buf, queue)
        return _Phase(W // COLS, groups, start)

    keys = functools.partial(head_matrix, k_hbm, k_s, S_K)
    vals = functools.partial(head_matrix, v_hbm, v_s, S_V)

    def start_qo(r, g, queue):
        src, dst, sem = (wq_hbm, wq_s, S_Q) if queue else (wo_hbm, wo_s, S_O)
        idx = (pl.ds(QO_GROUP * g, QO_GROUP), pl.ds(_aligned(QO_ROWS * r, QO_ROWS), QO_ROWS))
        copy(src.at[idx], dst.at[idx], sem, queue)

    def start_gu(r, c, queue):
        src, dst, sem = (wg_hbm, wg_s, S_G) if queue else (wu_hbm, wu_s, S_U)
        idx = (slice(None), pl.ds(_aligned(8 * r, 8), 8), pl.ds(COLS * c, COLS))
        copy(src.at[idx], dst.at[idx], sem, queue)

    DR = wd_hbm.shape[1]
    late = DR - LAST * LAST_ROWS
    S_DX, S_DL = S_D + late // 128, S_D + late // 128 + 1

    def start_down(r, _, queue):
        row = _aligned(8 * r, 8)
        if queue:
            sem = jnp.where(row < late, S_D + (row >> 7),
                            S_DL + ((row - late) >> (LAST_ROWS.bit_length() - 1)))
            idx = (pl.ds(0, WD_SLABS - 1), pl.ds(row, 8))
        else:
            sem = S_DX
            idx = (pl.ds(WD_SLABS - 1, 1), pl.ds(row, 8))
        copy(wd_hbm.at[idx], wd_s.at[idx], sem, queue)

    qo = _Phase(wq_hbm.shape[1] // QO_ROWS, QO_SLABS // QO_GROUP, start_qo)
    gu = _Phase(wg_hbm.shape[1] // 8, wg_hbm.shape[2] // COLS, start_gu)
    dn = _Phase(DR // 8, 1, start_down)

    QT = H * Dh // 128
    TR = wq_s.shape[1]
    assert TR & (TR - 1) == 0 and NBUF & (NBUF - 1) == 0

    def tile_rows(ref, row, n):
        return ref[row >> (TR.bit_length() - 1), pl.ds(_aligned(row & (TR - 1), n), n), :]

    def project(g):
        def band(b, acc):
            w = tile_rows(wq_s, (b * QT + 16 * g) * 8, 128)
            m = xc_s[pl.ds(pl.multiple_of(b * 8, 8), 8), :]
            return tuple(a + w[8 * j:8 * j + 8].astype(f32) * m for j, a in enumerate(acc))
        acc = lax.fori_loop(0, D // 8, band, tuple(jnp.zeros((8, 128), f32) for _ in range(16)),
                            unroll=2)
        for j in range(16):
            qt_s[:, pl.ds(_aligned((16 * g + j) * 128, 128), 128)] = jnp.broadcast_to(
                jnp.sum(acc[j], axis=0, keepdims=True), (8, 128))

    def scores(h):
        buf = h & (NBUF - 1)
        done(k_s.at[buf], S_K + buf)
        s = jnp.dot(q_s[h].astype(bf16), k_s[buf], preferred_element_type=f32) * Dh ** -0.5
        m = jnp.max(s, axis=-1, keepdims=True)
        e = jnp.exp(s - m)
        p_s[...] = e * (1.0 / jnp.sum(e, axis=-1, keepdims=True))

    def values(h):
        buf = h & (NBUF - 1)
        done(v_s.at[buf], S_V + buf)
        acc = [acc_s[:, t * 128:(t + 1) * 128] for t in range(DT)]
        for r in range(Dh // 16):
            a0 = jnp.zeros((8, 128), f32)
            a1 = jnp.zeros((8, 128), f32)
            for j in range(W // 128):
                vv = v_s[buf, r * 16:(r + 1) * 16, j * 128:(j + 1) * 128].astype(f32)
                pp = p_s[:, j * 128:(j + 1) * 128]
                a0 = a0 + vv[:8] * pp
                a1 = a1 + vv[8:] * pp
            o = (jnp.sum(a0, axis=-1, keepdims=True), jnp.sum(a1, axis=-1, keepdims=True))
            for t in range(DT):
                ww = tile_rows(wo_s, (h * Dh + r * 16) * DT + 16 * t, 16).astype(f32)
                for half in range(2):
                    band, col = divmod(2 * t + half, DT)
                    acc[col] = acc[col] + ww[8 * half:8 * half + 8] * o[band]
        for t in range(DT):
            acc_s[:, t * 128:(t + 1) * 128] = acc[t]

    lag = keys(0).slots
    lead = pl.cdiv(lag, qo.width) * qo.width
    x_cp = pltpu.make_async_copy(x_hbm, x_s, sems.at[S_X])
    wr_cp = pltpu.make_async_copy(wr_hbm, wr_s, sems.at[S_R])
    for i in range(lead):
        qo.start_slot(i, 1)
    x_cp.start()
    wr_cp.start()
    _stream(qo.slots - lead, qo, lead, qo)
    x_cp.wait()
    wr_cp.wait()
    x = x_s[0].astype(f32)
    xn = _layernorm(x).astype(bf16).astype(f32)
    for t in range(DT):
        xc_s[t * 128:(t + 1) * 128, :] = _column(xn[:, t * 128:(t + 1) * 128])
    acc_s[...] = jnp.zeros_like(acc_s)
    for i in range(lead):
        if i < lag:
            keys(0).start_slot(i, 1)
        qo.start_slot(qo.slots - lead + i, 0)

    def step(h, carry):
        @pl.when(h < H)
        def _():
            _stream(lag, vals(h), 0, keys(h))

        @pl.when(h == H)
        def _():
            _stream(lag, gu, lag, gu)

        @pl.when(h == 0)
        def _():
            done(wq_s, S_Q)

        @pl.when(h < 2)
        def _():
            project(2 * h)

        @pl.when(h >= 2)
        def _():
            scores(h - 2)

        @pl.when(h < H - 1)
        def _():
            _stream(lag, keys(h + 1), 0, vals(h))

        @pl.when(h == H - 1)
        def _():
            _stream(lag, gu, 0, vals(h))

        @pl.when(h == H)
        def _():
            _stream(gu.slots - 2 * lag, gu, 2 * lag, gu, lag)
            _stream(3 * lag - gu.slots, dn, 0, gu, gu.slots - lag)

        @pl.when(h == 0)
        def _():
            project(1)

        @pl.when(h == 1)
        def _():
            for c in range(H // 2):
                q2 = qt_s[:, c * 2 * Dh:(c + 1) * 2 * Dh]
                q_s[2 * c] = q2[:, :Dh]
                q_s[2 * c + 1] = q2[:, Dh:]
            done(wo_s, S_O)

        @pl.when(h >= 2)
        def _():
            values(h - 2)
        return carry

    lax.fori_loop(0, H + 1, step, 0)
    _stream(gu.slots - 2 * lag, dn, 3 * lag - gu.slots, gu, 2 * lag)
    scores(H - 1)

    def stream_down(lo, hi):
        both = max(min(hi, dn.slots - lag) - lo, 0)
        _stream(both, dn, lag + lo, dn, lo)
        _stream(hi - lo - both, None, 0, dn, lo + both)

    stream_down(0, 12)
    values(H - 1)

    hres = x + jnp.sum(acc_s[...], axis=0, keepdims=True)
    hn = _layernorm(hres)
    wr = wr_s[...].astype(f32).reshape(1, D)
    gate = jax.nn.sigmoid(jnp.sum(hn * wr, axis=-1, keepdims=True))
    hb = jnp.broadcast_to(hn, (8, D)).astype(bf16)

    stream_down(12, 36)
    done(wg_s, S_G)
    done(wu_s, S_U)
    act = []
    for c, (lo, hi) in enumerate(((36, 48), (48, dn.slots), (dn.slots, dn.slots))):
        cs = slice(c * DR, (c + 1) * DR)
        g = jnp.dot(hb, wg_s[:, :, cs].reshape(D, DR), preferred_element_type=f32)
        u = jnp.dot(hb, wu_s[:, :, cs].reshape(D, DR), preferred_element_type=f32)
        act.append((g * jax.nn.sigmoid(g) * u).astype(bf16))
        stream_down(lo, hi)

    def down(g, lo, hi):
        return jnp.dot(act[g][:, lo:hi], wd_s[g, lo:hi, :], preferred_element_type=f32)

    cols = [_column(act[g][:1, late:].astype(f32) * gate) for g in range(WD_SLABS - 1)]
    y = jnp.zeros((8, D), f32)
    for lo in range(0, late, 128):
        if lo + 128 == late:
            done(wd_s.at[WD_SLABS - 1], S_DX)
            y = y + down(WD_SLABS - 1, 0, DR)
        done(wd_s.at[pl.ds(0, WD_SLABS - 1), pl.ds(lo, 128)], S_D + lo // 128)
        for g in range(WD_SLABS - 1):
            y = y + down(g, lo, lo + 128)
    base = hres + (hn + y[:1] * gate)
    first = lax.broadcasted_iota(jnp.int32, (8, 128), 0) == 0
    a = [jnp.where(first, base[:, j * 128:(j + 1) * 128], 0.0) for j in range(DT)]
    for t in range(LAST):
        lo = late + LAST_ROWS * t
        done(wd_s.at[pl.ds(0, WD_SLABS - 1), pl.ds(lo, LAST_ROWS)], S_DL + t)
        for r in range(lo, lo + LAST_ROWS, 8):
            for g in range(WD_SLABS - 1):
                w = wd_s[g, r:r + 8, :].astype(f32)
                m = cols[g][r - late:r - late + 8]
                a = [a[j] + w[:, j * 128:(j + 1) * 128] * m for j in range(DT)]
    out = jnp.sum(jnp.concatenate(a, axis=1), axis=0, keepdims=True)
    o_ref[0] = out.astype(o_ref.dtype)


def _tiles(a):
    R, C = a.shape
    return a.reshape(R // 8, 8, C // 128, 128).transpose(0, 2, 1, 3).reshape(R * C // 128, 128)


def _slabs(a, n):
    return a.reshape(n, a.shape[0] // n, a.shape[1])


@jax.jit
def pallas_sequential_preLN__sliding_block_cached__moe_arch_mod__decode_kernel(
    A_x: jax.Array,
    A_k_cache: jax.Array,
    A_v_cache: jax.Array,
    A_wq: jax.Array,
    A_wo: jax.Array,
    B_x: jax.Array,
    B_w_r: jax.Array,
    B_w_gate: jax.Array,
    B_w_up: jax.Array,
    B_w_down: jax.Array,
):
    del B_x
    _, H, Sk, Dh = A_k_cache.shape
    D = A_x.shape[-1]
    W = min(4096, max(256, Sk // 4))
    kt = jnp.transpose(A_k_cache, (0, 1, 3, 2)).reshape(H * Dh, Sk)
    vt = jnp.transpose(A_v_cache, (0, 1, 3, 2)).reshape(H * Dh, Sk)
    wq, wo = _slabs(_tiles(A_wq), QO_SLABS), _slabs(_tiles(A_wo), QO_SLABS)
    wg, wu = _slabs(B_w_gate, GU_SLABS), _slabs(B_w_up, GU_SLABS)
    wd = _slabs(B_w_down, WD_SLABS)
    like = lambda a: pltpu.VMEM(a.shape, a.dtype)
    n_sems = 2 * NBUF + 6 + (wd.shape[1] - LAST * LAST_ROWS) // 128 + 1 + LAST
    return pl.pallas_call(
        _kernel,
        out_shape=jax.ShapeDtypeStruct(A_x.shape, A_x.dtype),
        in_specs=[pl.BlockSpec(memory_space=pl.ANY)] * 9,
        scratch_shapes=[
            like(A_x), like(B_w_r), like(wq), like(wo), like(wg), like(wu), like(wd),
            pltpu.VMEM((NBUF, Dh, W), A_k_cache.dtype),
            pltpu.VMEM((NBUF, Dh, W), A_v_cache.dtype),
            pltpu.VMEM((D, 128), f32),
            pltpu.VMEM((8, H * Dh), f32),
            pltpu.VMEM((H, 8, Dh), f32),
            pltpu.VMEM((8, W), f32),
            pltpu.VMEM((8, D), f32),
            pltpu.SemaphoreType.DMA((n_sems,)),
        ],
        compiler_params=pltpu.CompilerParams(
            vmem_limit_bytes=100 * 2**20,
            disable_bounds_checks=True,
            disable_semaphore_checks=True),
    )(A_x, kt, vt, wq, wo, B_w_r, wg, wu, wd)
```
